```python
import os as _os
_os.environ.setdefault("JAX_PLATFORMS", "cpu")
import jax
import jax.numpy as jnp

def _softmax(x, axis=-1):
    return jax.nn.softmax(x, axis=axis)
def _gelu(x):
    return jax.nn.gelu(x, approximate=True)
def _silu(x):
    return jax.nn.silu(x)
def _sigmoid(x):
    return jax.nn.sigmoid(x)
def _layernorm(x, axis=-1, eps=1e-5):
    m = jnp.mean(x, axis=axis, keepdims=True)
    v = jnp.var(x, axis=axis, keepdims=True)
    return (x - m) / jnp.sqrt(v + eps)
def _scatter_add(tgt, idx, src, axis=0):
    return tgt.at[idx].add(src)
def _segment_sum(src, seg, n):
    return jax.ops.segment_sum(src, seg, n)
class _Rng:
    def __init__(self, key):
        self._k = key
    def _next(self):
        self._k, sub = jax.random.split(self._k)
        return sub
    def normal(self, shape):
        return jax.random.normal(self._next(), shape, dtype=jnp.bfloat16)
    def randint(self, lo, hi, shape):
        return jax.random.randint(self._next(), shape, lo, hi, dtype=jnp.int32)
    def uniform(self, shape, lo=0.0, hi=1.0):
        return jax.random.uniform(self._next(), shape, jnp.bfloat16, lo, hi)
    def permutation(self, n):
        return jax.random.permutation(self._next(), n)


kernel_name = 'standalone__mha_softmax__near_ridge'

def setup_inputs():
    _rng = _Rng(jax.random.key(int.from_bytes(__import__("os").urandom(4), "little")))
    _w = (lambda a: (lambda t: t.astype(jnp.bfloat16) if jnp.issubdtype(t.dtype, jnp.floating) else t)(jnp.asarray(a)))
    B, H, Sq, Sk, D = 8, 32, 496, 512, 192
    return {
        "q": _w((lambda *s: _rng.normal(s) * 0.05)(B, H, Sq, D)),
        "k": _w((lambda *s: _rng.normal(s) * 3.2)(B, H, Sk, D)),
        "v": _w((lambda *s: _rng.normal(s) * 0.05)(B, H, Sk, D)),
    }

def reference(q, k, v):
    scale = q.shape[-1] ** -0.5
    scores = jnp.einsum("bhqd,bhkd->bhqk", q, k) * scale
    p = _softmax(scores, axis=-1)
    return jnp.einsum("bhqk,bhkd->bhqd", p, v)
```

```python
import jax
import jax.numpy as jnp
import jax.experimental.pallas as pl
import jax.experimental.pallas.tpu as pltpu

_HB = 8


def _attn_kernel(qt_ref, kt_ref, vt_ref, ot_ref):
    scale = qt_ref.shape[-2] ** -0.5
    for h in range(qt_ref.shape[1]):
        qt = qt_ref[0, h]
        kt = kt_ref[0, h]
        vt = vt_ref[0, h]
        st = jax.lax.dot_general(kt, qt, (((0,), (0,)), ((), ())),
                                 preferred_element_type=jnp.float32)
        m = jnp.max(st, axis=0, keepdims=True)
        p = jnp.exp((st - m) * scale)
        l = jnp.sum(p, axis=0, keepdims=True)
        ot = jnp.dot(vt, p.astype(jnp.bfloat16), preferred_element_type=jnp.float32)
        ot_ref[0, h] = (ot / l).astype(ot_ref.dtype)


@jax.jit
def pallas_standalone__mha_softmax__near_ridge_kernel(
    q: jax.Array,
    k: jax.Array,
    v: jax.Array,
):
    B, H, Sq, D = q.shape
    Sk = k.shape[2]
    hb = _HB if H % _HB == 0 else 1
    qt, kt, vt = (jnp.swapaxes(x, 2, 3) for x in (q, k, v))
    ot = pl.pallas_call(
        _attn_kernel,
        grid=(B, H // hb),
        in_specs=[
            pl.BlockSpec((1, hb, D, Sq), lambda b, h: (b, h, 0, 0)),
            pl.BlockSpec((1, hb, D, Sk), lambda b, h: (b, h, 0, 0)),
            pl.BlockSpec((1, hb, D, Sk), lambda b, h: (b, h, 0, 0)),
        ],
        out_specs=pl.BlockSpec((1, hb, D, Sq), lambda b, h: (b, h, 0, 0)),
        out_shape=jax.ShapeDtypeStruct(qt.shape, q.dtype),
        compiler_params=pltpu.CompilerParams(
            dimension_semantics=("parallel", "parallel"),
            vmem_limit_bytes=64 * 1024 * 1024),
    )(qt, kt, vt)
    return jnp.swapaxes(ot, 2, 3)
```

```python
import math

import jax
import jax.numpy as jnp
import jax.experimental.pallas as pl
import jax.experimental.pallas.tpu as pltpu

_HB = 8


def _attn_kernel(qt_ref, kt_ref, vt_ref, ot_ref):
    hb, D = qt_ref.shape[1], qt_ref.shape[2]
    c2 = (D ** -0.5) * math.log2(math.e)

    def qk(h):
        return jax.lax.dot_general(kt_ref[0, h], qt_ref[0, h], (((0,), (0,)), ((), ())),
                                   preferred_element_type=jnp.float32)

    st_next = qk(0)
    for h in range(hb):
        st = st_next
        if h + 1 < hb:
            st_next = qk(h + 1)
        m = jnp.max(st, axis=0, keepdims=True)
        p = jnp.exp2((st - m) * c2)
        l = jnp.sum(p, axis=0, keepdims=True)
        ot = jnp.dot(vt_ref[0, h], p.astype(jnp.bfloat16),
                     preferred_element_type=jnp.float32)
        ot_ref[0, h] = (ot * (1.0 / l)).astype(ot_ref.dtype)


@jax.jit
def pallas_standalone__mha_softmax__near_ridge_kernel(
    q: jax.Array,
    k: jax.Array,
    v: jax.Array,
):
    B, H, Sq, D = q.shape
    Sk = k.shape[2]
    hb = _HB if H % _HB == 0 else 1
    qt, kt, vt = (jnp.swapaxes(x, 2, 3) for x in (q, k, v))
    ot = pl.pallas_call(
        _attn_kernel,
        grid=(B, H // hb),
        in_specs=[
            pl.BlockSpec((1, hb, D, Sq), lambda b, h: (b, h, 0, 0)),
            pl.BlockSpec((1, hb, D, Sk), lambda b, h: (b, h, 0, 0)),
            pl.BlockSpec((1, hb, D, Sk), lambda b, h: (b, h, 0, 0)),
        ],
        out_specs=pl.BlockSpec((1, hb, D, Sq), lambda b, h: (b, h, 0, 0)),
        out_shape=jax.ShapeDtypeStruct(qt.shape, q.dtype),
        compiler_params=pltpu.CompilerParams(
            dimension_semantics=("parallel", "parallel"),
            vmem_limit_bytes=96 * 1024 * 1024),
    )(qt, kt, vt)
    return jnp.swapaxes(ot, 2, 3)
```
